```python
import jax
import jax.numpy as jnp

def _softmax(x, axis=-1):
    return jax.nn.softmax(x, axis=axis)
def _gelu(x):
    return jax.nn.gelu(x, approximate=True)
def _silu(x):
    return jax.nn.silu(x)
def _sigmoid(x):
    return jax.nn.sigmoid(x)
def _layernorm(x, axis=-1, eps=1e-5):
    m = jnp.mean(x, axis=axis, keepdims=True)
    v = jnp.var(x, axis=axis, keepdims=True)
    return (x - m) / jnp.sqrt(v + eps)
def _scatter_add(tgt, idx, src, axis=0):
    return tgt.at[idx].add(src)
def _segment_sum(src, seg, n):
    return jax.ops.segment_sum(src, seg, n)
class _Rng:
    def __init__(self, key):
        self._k = key
    def _next(self):
        self._k, sub = jax.random.split(self._k)
        return sub
    def normal(self, shape):
        return jax.random.normal(self._next(), shape, dtype=jnp.bfloat16)
    def randint(self, lo, hi, shape):
        return jax.random.randint(self._next(), shape, lo, hi, dtype=jnp.int32)
    def uniform(self, shape, lo=0.0, hi=1.0):
        return jax.random.uniform(self._next(), shape, jnp.bfloat16, lo, hi)
    def permutation(self, n):
        return jax.random.permutation(self._next(), n)


kernel_name = 'standalone__batchnorm__sampling'

def setup_inputs():
    _rng = _Rng(jax.random.key(int.from_bytes(__import__("os").urandom(4), "little")))
    _w = (lambda a: (lambda t: t.astype(jnp.bfloat16) if jnp.issubdtype(t.dtype, jnp.floating) else t)(jnp.asarray(a)))
    B, S, C = 1024, 32, 576
    K = 3
    return {
        "x": _w((lambda *s: _rng.normal(s) * 0.05)(B, S, C)),
        "w": _w((lambda *s: _rng.normal(s) * 0.05)(K, C, C) * (1.0 / (K * C) ** 0.5)),
        "mean": _w((lambda *s: _rng.normal(s) * 0.05)(C) * 0.1),
        "var": _w(jnp.abs((lambda *s: _rng.normal(s) * 0.05)(C)) + 0.5),
        "g": _w((lambda *s: _rng.normal(s) * 0.05)(C) + 1.0),
        "b": _w((lambda *s: _rng.normal(s) * 0.05)(C) * 0.1),
    }

def reference(x, w, mean, var, g, b):
    K = 3
    P = K // 2
    S = x.shape[1]
    xp = jnp.pad(x, ((0, 0), (P, P), (0, 0)))
    y = sum(jnp.einsum('bsc,cd->bsd', xp[:, k:k + S, :], w[k]) for k in range(K))
    inv_std = 1.0 / jnp.sqrt(var + 1e-5)
    y = (y - mean) * (g * inv_std) + b
    return _silu(y)
```

```python
import jax
import jax.numpy as jnp
import numpy as np
import jax.experimental.pallas as pl
import jax.experimental.pallas.tpu as pltpu

NB = 128

def _kernel(x_ref, w_ref, mean_ref, var_ref, g_ref, b_ref, o_ref, gt_ref, bias_ref, u_ref):
    S, C, nb = x_ref.shape
    f32 = jnp.float32

    @pl.when(pl.program_id(0) == 0)
    def _():
        f = lambda r: r[...].astype(f32)
        scale = 0.5 * f(g_ref) * jax.lax.rsqrt(f(var_ref) + 1e-5)
        bias = 0.5 * f(b_ref) - f(mean_ref) * scale
        bias_ref[...] = jnp.broadcast_to(bias, (nb, C)).T
        w0 = w_ref[0].astype(f32) * scale
        w1 = w_ref[1].astype(f32) * scale
        w2 = w_ref[2].astype(f32) * scale
        gs = [w0 * 0.25,
              (w0 + w1 + w2) * (-1.0 / 6),
              (w0 - w1 + w2) * (-1.0 / 6),
              w0 * (1 / 24) + w1 * (1 / 12) + w2 * (1 / 6),
              w0 * (1 / 24) - w1 * (1 / 12) + w2 * (1 / 6),
              w2]
        for j in range(6):
            gt_ref[j] = gs[j].T.astype(jnp.bfloat16)

    def row(s):
        if s < 0 or s >= S:
            return jnp.zeros((C, nb), f32)
        return x_ref[s].astype(f32)

    for t in range(S // 4):
        d0, d1, d2, d3, d4, d5 = [row(4 * t - 1 + i) for i in range(6)]
        t0 = d4 - 4 * d2
        t1 = d3 - 4 * d1
        t2 = d4 - d2
        e = d1 - d3
        t3 = -2 * e
        us = [4 * (d0 - d2) + t2, t0 + t1, t0 - t1, t2 + t3, t2 - t3, 4 * e + (d5 - d3)]
        m = [jnp.dot(gt_ref[j], us[j].astype(jnp.bfloat16), preferred_element_type=f32) for j in range(6)]
        m1 = m[1] + bias_ref[...]
        s0 = m1 + m[2]
        s1 = m1 - m[2]
        s2 = m[3] + m[4]
        s3 = m[3] - m[4]
        ys = [m[0] + s0 + s2, s1 + 2 * s3, s0 + 4 * s2, s1 + 8 * s3 + m[5]]
        for r in range(4):
            h = ys[r]
            o_ref[4 * t + r] = (h * jnp.tanh(h) + h).astype(o_ref.dtype)

@jax.jit
def pallas_standalone__batchnorm__sampling_kernel(x, w, mean, var, g, b):
    B, S, C = x.shape
    xt = jnp.transpose(x, (1, 2, 0))
    vec = pl.BlockSpec((1, C), lambda i: (0, 0))
    out = pl.pallas_call(
        _kernel,
        grid=(B // NB,),
        in_specs=[pl.BlockSpec((S, C, NB), lambda i: (0, 0, i)),
                  pl.BlockSpec((3, C, C), lambda i: (0, 0, 0)), vec, vec, vec, vec],
        out_specs=pl.BlockSpec((S, C, NB), lambda i: (0, 0, i)),
        out_shape=jax.ShapeDtypeStruct((S, C, B), x.dtype),
        scratch_shapes=[pltpu.VMEM((6, C, C), jnp.bfloat16), pltpu.VMEM((C, NB), jnp.float32), pltpu.VMEM((6, C, NB), jnp.bfloat16)],
        compiler_params=pltpu.CompilerParams(dimension_semantics=("arbitrary",), vmem_limit_bytes=100 * 2**20),
    )(xt, w, mean.reshape(1, C), var.reshape(1, C), g.reshape(1, C), b.reshape(1, C))
    return jnp.transpose(out, (2, 0, 1))
```

```python
import jax
import jax.numpy as jnp
import jax.experimental.pallas as pl
import jax.experimental.pallas.tpu as pltpu

NB = 128
U32 = 1
P29 = 1
ORD = (5, 0, 1, 2, 3, 4)

def _kernel(x_hbm, w_hbm, mean_hbm, var_hbm, g_hbm, b_hbm, o_hbm,
            xbuf, obuf, wbuf, vb0, vb1, vb2, vb3, g0, g1, g2, g3, g4, g5, bias_ref, xsem, osem, wsem, vsem):
    S, C, B = x_hbm.shape
    nb = NB
    NBLK = B // nb
    T = S // 4
    f32 = jnp.float32
    bf16 = jnp.bfloat16
    KT = (C + 127) // 128
    CH = C - 64

    def xrows(gi):
        if gi == 0:
            return 0, 1
        lo = 4 * (gi - 1) + 1
        return lo, min(4, S - lo)

    def xcopy(n, slot, gi):
        lo, cnt = xrows(gi)
        return pltpu.make_async_copy(
            x_hbm.at[pl.ds(lo, cnt), :, pl.ds(pl.multiple_of(n * nb, nb), nb)],
            xbuf.at[slot, pl.ds(lo, cnt)], xsem.at[slot * (T + 1) + gi])

    def ocopy(n, slot, t):
        return pltpu.make_async_copy(
            obuf.at[slot, pl.ds(4 * t, 4)],
            o_hbm.at[pl.ds(4 * t, 4), :, pl.ds(pl.multiple_of(n * nb, nb), nb)],
            osem.at[slot * T + t])

    def wcopy(k):
        kk = min(128, C - 128 * k)
        return pltpu.make_async_copy(w_hbm.at[:, pl.ds(128 * k, kk), :], wbuf.at[:, pl.ds(128 * k, kk), :], wsem.at[k])

    vbuf = (vb0, vb1, vb2, vb3)
    vcopies = [pltpu.make_async_copy(r, vbuf[i], vsem.at[i]) for i, r in enumerate((mean_hbm, var_hbm, g_hbm, b_hbm))]
    for c in vcopies:
        c.start()
    korder = [KT - 1] + list(range(KT - 1))
    wcopy(korder[0]).start()
    xcopy(0, 0, 0).start()
    xcopy(0, 0, 1).start()
    for k in korder[1:]:
        wcopy(k).start()

    for c in vcopies:
        c.wait()
    f = lambda i: vbuf[i][...].astype(f32).reshape(1, C)
    scale = 0.5 * f(2) * jax.lax.rsqrt(f(1) + 1e-5)
    bias = 0.5 * f(3) - f(0) * scale
    bias_ref[...] = jnp.broadcast_to(bias, (nb, C)).T

    def combos(w0, w1, w2):
        a = w0 + w2
        q = w0 * (1 / 24) + w2 * (1 / 6)
        r = w1 * (1 / 12)
        return [w0 * 0.25, (a + w1) * (-1.0 / 6), (a - w1) * (-1.0 / 6), q + r, q - r, w2]

    def put(j, k, val):
        v = val.astype(bf16)
        if U32:
            v = pltpu.bitcast(v, jnp.uint32)
        gts[j][:, 128 * k:128 * k + v.shape[1]] = v

    gts = (g0, g1, g2, g3, g4, g5)
    beta = (6.0, -4.0, -4.0, 1.0, 1.0, 0.0)
    for k in korder:
        wcopy(k).wait()
        kk = min(128, C - 128 * k)
        ws = [wbuf[i, 128 * k:128 * k + kk, :].astype(f32) * scale for i in range(3)]
        if kk == 128:
            gs = combos(*[v.T for v in ws])
            for j in range(6):
                put(j, k, gs[j])
        else:
            gs = combos(*ws)
            z = jnp.zeros_like(gs[0])
            for j in range(6):
                if P29:
                    if j == 0:
                        continue
                    ext = gs[0] * (-beta[j] / beta[0]) if j < 5 else z
                else:
                    ext = z
                tt = jnp.concatenate([gs[j], ext], 0).T
                put(j, k, tt if gts[j].shape[1] == 128 * KT else tt[:, :kk])

    def transform(slot, t, ub):
        def row(s):
            if s < 0 or s >= S:
                return jnp.zeros((C, nb), f32)
            return xbuf[slot, s].astype(f32)
        d0, d1, d2, d3, d4, d5 = [row(4 * t - 1 + i) for i in range(6)]
        t0 = d4 - 4 * d2
        t1 = d3 - 4 * d1
        t2 = d4 - d2
        e = d1 - d3
        t3 = -2 * e
        us = [4 * (d0 - d2) + t2, t0 + t1, t0 - t1, t2 + t3, t2 - t3, 4 * e + (d5 - d3)]
        return us

    def getg(j):
        v = gts[j][...]
        return pltpu.bitcast(v, bf16) if U32 else v

    def rhs32(j, us):
        if P29:
            if j == 0:
                return us[0][:CH]
            if j < 5:
                return jnp.concatenate([us[j], us[0][CH:]], 0)
        return us[j]

    def mm(j, us):
        r = rhs32(j, us).astype(bf16)
        return jnp.dot(getg(j), r, preferred_element_type=f32)

    pl.delay(1)
    for gi in range(2, T + 1):
        xcopy(0, 0, gi).start()
    def block(n, carry):
        slot = jax.lax.rem(n, 2)

        @pl.when(n >= 2)
        def _():
            for t in range(T):
                ocopy(n - 2, slot, t).wait()

        for t in range(T):
            if t == 0:
                xcopy(n, slot, 0).wait()
            xcopy(n, slot, t + 1).wait()
            us = transform(slot, t, None)
            md = {j: mm(j, us) for j in ORD}; m = [md[j] for j in range(6)]
            m1 = m[1] + bias_ref[...]
            s0 = m1 + m[2]
            s1 = m1 - m[2]
            s2 = m[3] + m[4]
            s3 = m[3] - m[4]
            ys = [m[0] + s0 + s2, s1 + 2 * s3, s0 + 4 * s2, s1 + 8 * s3 + m[5]]
            for r in range(4):
                h = ys[r]
                obuf[slot, 4 * t + r] = (h * jnp.tanh(h) + h).astype(obuf.dtype)
            ocopy(n, slot, t).start()
            @pl.when(n + 1 < NBLK)
            def _():
                for gi in ((0, 1) if t == 0 else (t + 1,)):
                    xcopy(n + 1, 1 - slot, gi).start()

        return carry

    jax.lax.fori_loop(0, NBLK, block, 0)
    for n in range(NBLK - 2, NBLK):
        for t in range(T):
            ocopy(n, n % 2, t).wait()

@jax.jit
def pallas_standalone__batchnorm__sampling_kernel(x, w, mean, var, g, b):
    B, S, C = x.shape
    xt = jnp.transpose(x, (1, 2, 0))
    T = S // 4
    gdt, gr = (jnp.uint32, C // 2) if U32 else (jnp.bfloat16, C)
    kws = [C - 64] + [C + 64] * 4 + [C] if P29 else [C] * 6
    anyspec = pl.BlockSpec(memory_space=pl.ANY)
    out = pl.pallas_call(
        _kernel,
        in_specs=[anyspec] * 6,
        out_specs=anyspec,
        out_shape=jax.ShapeDtypeStruct((S, C, B), x.dtype),
        scratch_shapes=[pltpu.VMEM((2, S, C, NB), jnp.bfloat16), pltpu.VMEM((2, S, C, NB), jnp.bfloat16),
                        pltpu.VMEM((3, C, C), jnp.bfloat16), *[pltpu.VMEM((C,), jnp.bfloat16)] * 4,
                        *[pltpu.VMEM((gr, kw), gdt) for kw in kws],
                        pltpu.VMEM((C, NB), jnp.float32),
                        pltpu.SemaphoreType.DMA((2 * (T + 1),)), pltpu.SemaphoreType.DMA((2 * T,)),
                        pltpu.SemaphoreType.DMA((5,)), pltpu.SemaphoreType.DMA((4,))],
        compiler_params=pltpu.CompilerParams(vmem_limit_bytes=100 * 2**20, flags={"XLA_TPU_RESCHEDULE_DMA_DONES": True}),
    )(xt, w, mean, var, g, b)
    return jnp.transpose(out, (2, 0, 1))
```
